```python
import jax
import jax.numpy as jnp

def _softmax(x, axis=-1):
    return jax.nn.softmax(x, axis=axis)

def _gelu(x):
    return jax.nn.gelu(x, approximate=True)

def _silu(x):
    return jax.nn.silu(x)

def _sigmoid(x):
    return jax.nn.sigmoid(x)

def _layernorm(x, axis=-1, eps=1e-05):
    m = jnp.mean(x, axis=axis, keepdims=True)
    v = jnp.var(x, axis=axis, keepdims=True)
    return (x - m) / jnp.sqrt(v + eps)

def _scatter_add(tgt, idx, src, axis=0):
    return tgt.at[idx].add(src)

def _segment_sum(src, seg, n):
    return jax.ops.segment_sum(src, seg, n)

class _Rng:

    def __init__(self, key):
        self._k = key

    def _next(self):
        self._k, sub = jax.random.split(self._k)
        return sub

    def normal(self, shape):
        return jax.random.normal(self._next(), shape, dtype=jnp.bfloat16)

    def randint(self, lo, hi, shape):
        return jax.random.randint(self._next(), shape, lo, hi, dtype=jnp.int32)

    def uniform(self, shape, lo=0.0, hi=1.0):
        return jax.random.uniform(self._next(), shape, jnp.bfloat16, lo, hi)

    def permutation(self, n):
        return jax.random.permutation(self._next(), n)
kernel_name = 'interleave_layers__linear_kernel_hedgehog__memory_aug_recurrent_mem_tr__prompt'

def setup_inputs():
    _rng = _Rng(jax.random.key(int.from_bytes(__import__("os").urandom(4), "little")))
    _w = lambda a: (lambda t: t.astype(jnp.bfloat16) if jnp.issubdtype(t.dtype, jnp.floating) else t)(jnp.asarray(a))

    def _A_setup():
        B, S, D, H = (1, 2048, 640, 32)
        Dh = D // H
        return {'x': _w((lambda *s: _rng.normal(s) * 0.05)(B, S, D)), 'wqkv': _w((lambda *s: _rng.normal(s) * 0.05)(D, 3 * D)), 'w_phi': _w((lambda *s: _rng.normal(s) * 0.05)(H, Dh, Dh) * Dh ** (-0.5)), 'wo': _w((lambda *s: _rng.normal(s) * 0.05)(D, D))}
    _A_in = _A_setup()

    def _B_setup():
        B, S, Dm = (1, 2048, 640)
        H, Dh = (32, 192)
        M, seg = (8, 32)
        seg = min(seg, S)
        S = S // seg * seg
        return {'x': _w((lambda *s: _rng.normal(s) * 0.05)(B, S, Dm)), 'mem0': _w((lambda *s: _rng.normal(s) * 0.05)(B, M, Dm)), 'Wq': _w((lambda *s: _rng.normal(s) * 0.05)(Dm, H, Dh) * Dm ** (-0.5)), 'Wk': _w((lambda *s: _rng.normal(s) * 0.05)(Dm, H, Dh) * Dm ** (-0.5)), 'Wv': _w((lambda *s: _rng.normal(s) * 0.05)(Dm, H, Dh) * Dm ** (-0.5)), 'Wo': _w((lambda *s: _rng.normal(s) * 0.05)(H, Dh, Dm) * (H * Dh) ** (-0.5)), 'seg_len': seg}
    _B_in = _B_setup()
    return {'A_x': _A_in['x'], 'A_wqkv': _A_in['wqkv'], 'A_w_phi': _A_in['w_phi'], 'A_wo': _A_in['wo'], 'B_x': _B_in['x'], 'B_mem0': _B_in['mem0'], 'B_Wq': _B_in['Wq'], 'B_Wk': _B_in['Wk'], 'B_Wv': _B_in['Wv'], 'B_Wo': _B_in['Wo'], 'B_seg_len': _B_in['seg_len']}

def reference(A_x, A_wqkv, A_w_phi, A_wo, B_x, B_mem0, B_Wq, B_Wk, B_Wv, B_Wo, B_seg_len):

    def _A_ref(x, wqkv, w_phi, wo):
        B, S, D = x.shape
        H = 32
        Dh = D // H
        qkv = (lambda x, *d: x.transpose(*d))((x @ wqkv).reshape(B, S, 3, H, Dh), 2, 0, 3, 1, 4)
        q, k, v = (qkv[0], qkv[1], qkv[2])
        pq = jnp.einsum('bhsd,hdf->bhsf', q, w_phi)
        pk = jnp.einsum('bhsd,hdf->bhsf', k, w_phi)
        phi_q = jnp.concatenate([_softmax(pq, axis=-1), _softmax(-pq, axis=-1)], axis=-1)
        phi_k = jnp.concatenate([_softmax(pk, axis=-1), _softmax(-pk, axis=-1)], axis=-1)
        kv = jnp.einsum('bhsf,bhsd->bhfd', phi_k, v)
        z = jnp.einsum('bhsf->bhf', phi_k)
        num = jnp.einsum('bhqf,bhfd->bhqd', phi_q, kv)
        den = jnp.einsum('bhqf,bhf->bhq', phi_q, z)[..., None] + 1e-06
        o = num / den
        return (lambda x, *d: x.transpose(*d))(o, 0, 2, 1, 3).reshape(B, S, D) @ wo

    def _B_ref(x, mem0, Wq, Wk, Wv, Wo, seg_len):
        B, S, Dm = x.shape
        H, Dh = (Wq.shape[1], Wq.shape[2])
        M = mem0.shape[1]
        scale = Dh ** (-0.5)
        n_seg = S // seg_len
        L = M + seg_len
        idx = jnp.arange(L)
        mask = (idx[:, None] < M) | (idx[:, None] >= idx[None, :])
        mem = mem0
        outs = []
        for s in range(n_seg):
            xs = x[:, s * seg_len:(s + 1) * seg_len, :].copy()
            h = jnp.concatenate([mem, xs], axis=1)
            q = jnp.einsum('btd,dhe->bhte', h, Wq)
            k = jnp.einsum('btd,dhe->bhte', h, Wk)
            v = jnp.einsum('btd,dhe->bhte', h, Wv)
            scores = jnp.einsum('bhqe,bhke->bhqk', q, k) * scale
            scores = jnp.where(mask[None, None], scores, -1000000000.0)
            p = _softmax(scores, axis=-1)
            o = jnp.einsum('bhqk,bhke->bhqe', p, v)
            o = jnp.einsum('bhte,hed->btd', o, Wo)
            mem = o[:, :M, :].copy()
            outs.append(o[:, M:, :])
        return jnp.concatenate(outs, axis=1)
    x = A_x
    x = x + _A_ref(_layernorm(x, axis=-1), A_wqkv, A_w_phi, A_wo)
    x = x + _B_ref(_layernorm(x, axis=-1), B_mem0, B_Wq, B_Wk, B_Wv, B_Wo, B_seg_len)
    x = x + _A_ref(_layernorm(x, axis=-1), A_wqkv, A_w_phi, A_wo)
    x = x + _B_ref(_layernorm(x, axis=-1), B_mem0, B_Wq, B_Wk, B_Wv, B_Wo, B_seg_len)
    return x
```

```python
import functools

import jax
import jax.numpy as jnp
from jax import lax
import jax.experimental.pallas as pl
import jax.experimental.pallas.tpu as pltpu

F32 = jnp.float32
BF16 = jnp.bfloat16
NT = (((1,), (1,)), ((), ()))
HA = 32
NC = 8
WARM = 3


def _dot(a, b):
    return jnp.dot(a, b, preferred_element_type=F32)


def _dot_nt(a, b):
    return lax.dot_general(a, b, NT, preferred_element_type=F32)


def _iota(shape, d):
    return lax.broadcasted_iota(jnp.int32, shape, d)


def _kernel(x_ref, wqkv_ref, phit_ref, wo_ref, mem0_ref, wq_hbm, wk_hbm, wv_hbm, wo_hbm,
            out_ref, xs, hs, wq, wk, wv, wob, wqt, wkt, wot, sems, *, seg, dhb):
    S, D = xs.shape
    HD = wq.shape[0]
    M = mem0_ref.shape[0]
    dha = D // HA
    gw = dha * 8
    ng = HA // 8
    nseg = S // seg
    nj = nseg // NC
    R = NC * seg
    nb = NC // 2
    TB, MB = 2 * seg, 2 * M
    KB = TB + MB
    PW = 2 * dhb
    npair = HD // PW
    assert dhb == 192 and M == 8 and seg % 16 == 0 and KB <= 128
    scale = dhb ** -0.5

    copies = [pltpu.make_async_copy(s, d, sems.at[i])
              for i, (s, d) in enumerate(((wk_hbm, wk), (wv_hbm, wv), (wq_hbm, wq), (wo_hbm, wob)))]
    for c in copies:
        c.start()

    def seg_rows(i):
        j, c = i // NC, i % NC
        return (pl.ds(pl.multiple_of(i * seg, seg), seg),
                pl.ds(pl.multiple_of((c * nj + j) * seg, seg), seg))

    @pl.loop(0, nseg)
    def _(i):
        mine, orig = seg_rows(i)
        xs[mine, :] = x_ref[orig, :].astype(F32)

    def head_of(n):
        g = sum((n >= k * gw).astype(jnp.int32) for k in range(1, ng))
        return g * 8 + (n & 7)

    def same_head(n, r):
        lo = head_of(n) * dha
        return (r >= lo) & (r < lo + dha)

    bdt = jnp.where(same_head(_iota((D, D), 0), _iota((D, D), 1)),
                    phit_ref[...].astype(F32), 0.0).astype(BF16)
    wqt[...] = _dot_nt(bdt, wqkv_ref[:, 0:D]).astype(BF16)
    wkt[...] = _dot_nt(bdt, wqkv_ref[:, D:2 * D]).astype(BF16)
    wot[...] = wo_ref[...].astype(F32).T.astype(BF16)

    def layernorm():
        T = 256

        @pl.loop(0, S // T)
        def _(i):
            r = pl.ds(pl.multiple_of(i * T, T), T)
            x = xs[r, :]
            d = x - jnp.mean(x, axis=-1, keepdims=True)
            v = jnp.mean(d * d, axis=-1, keepdims=True)
            hs[r, :] = (d * lax.rsqrt(v + 1e-5)).astype(BF16)

    def tiles(wt, T):
        proj = lambda i: _dot_nt(wt[...], hs[i * T:(i + 1) * T, :])
        nxt = proj(0)
        for i in range(S // T):
            cur, nxt = nxt, (proj(i + 1) if i + 1 < S // T else None)
            yield slice(i * T, (i + 1) * T), features(cur)

    def features(p):
        p = p.reshape(ng, dha, 8, p.shape[1])
        ep = jnp.exp(p - jnp.max(p, axis=1, keepdims=True))
        en = jnp.exp(jnp.min(p, axis=1, keepdims=True) - p)
        ep = ep * (1.0 / jnp.sum(ep, axis=1, keepdims=True))
        en = en * (1.0 / jnp.sum(en, axis=1, keepdims=True))
        return ep, en

    def layer_a():
        T = 256

        def body(kh, zs, mt):
            kh[...] = jnp.zeros_like(kh)
            zs[...] = jnp.zeros_like(zs)

            for r, (ep, en) in tiles(wkt, T):
                h = hs[r, :]
                phi = jnp.concatenate([ep.reshape(D, T), en.reshape(D, T)], axis=0)
                zs[...] += sum(phi[:, k * 128:(k + 1) * 128] for k in range(T // 128))
                kh[...] += _dot(phi.astype(BF16), h)

            z = jnp.sum(zs[...], axis=-1, keepdims=True)
            zs[...] = jnp.broadcast_to(z, zs.shape)
            keep = same_head(_iota((D, D), 0), _iota((D, D), 1))
            for s in range(2):
                kv = _dot(kh[s * D:(s + 1) * D, :].astype(BF16), wqkv_ref[:, 2 * D:3 * D])
                kv = jnp.where(keep, kv, 0.0).astype(BF16)
                mt[:, s * D:(s + 1) * D] = _dot_nt(wot[...], kv).astype(BF16)

            for r, (ep, en) in tiles(wqt, T):
                zt = jnp.concatenate([zs[...]] * (T // 128), axis=1)
                den = jnp.sum(ep * zt[:D].reshape(ng, dha, 8, T) + en * zt[D:].reshape(ng, dha, 8, T),
                              axis=1, keepdims=True)
                inv = 1.0 / (den + 1e-6)
                phi = jnp.concatenate([(ep * inv).reshape(D, T), (en * inv).reshape(D, T)], axis=0)
                xs[r, :] += _dot(mt[...], phi.astype(BF16)).T

        pl.run_scoped(body, pltpu.VMEM((2 * D, D), F32), pltpu.VMEM((2 * D, 128), F32),
                      pltpu.VMEM((D, 2 * D), BF16))

    def attend(q, kall, vall, km, vm, j, lanes, mask):
        n = q.shape[0] // nb
        low = _iota((1, 128), 1) < dhb - 128
        mid = q[:, 128:256]
        qa = jnp.concatenate([q[:, :128], jnp.where(low, mid, 0.0)], axis=1).astype(BF16)
        qb = jnp.concatenate([jnp.where(low, 0.0, mid), q[:, 256:]], axis=1).astype(BF16)
        s = []
        for b in range(nb):
            k = jnp.concatenate([kall[j * nb + b, :, lanes], km[b]], axis=0)
            s.append(_dot_nt(qa[b * n:(b + 1) * n], k[:, :256]))
            s.append(_dot_nt(qb[b * n:(b + 1) * n], k[:, 128:]))
        return lambda: finish(s, vall, vm, j, lanes, mask, low)

    def finish(s, vall, vm, j, lanes, mask, low):
        s = jnp.where(mask[None], jnp.stack(s) * scale, -1e9)
        e = jnp.exp(s - jnp.max(s, axis=-1, keepdims=True))
        p = (e * (1.0 / jnp.sum(e, axis=-1, keepdims=True))).astype(BF16)
        o = []
        for b in range(nb):
            v = jnp.concatenate([vall[j * nb + b, :, lanes], vm[b]], axis=0)
            n = p.shape[1]
            om = _dot(p[2 * b:2 * b + 2].reshape(2 * n, KB), v[:, 128:256])
            o.append(jnp.concatenate(
                [_dot(p[2 * b], v[:, :128]), jnp.where(low, om[:n], om[n:]),
                 _dot(p[2 * b + 1], v[:, 256:])], axis=1))
        return jnp.concatenate(o, axis=0).astype(BF16)

    def layer_b(first):
        CH = 1536

        def body(kall, vall, mems, kmem, vmem):
            ns = jax.named_scope("kv"); ns.__enter__()
            for dst, w, cp in ((kall, wk, 0), (vall, wv, 1)):
                if first:
                    copies[cp].wait()

                @pl.loop(0, nj)
                def _(j):
                    h = hs[pl.ds(pl.multiple_of(j * R, R), R), :]
                    for c in range(HD // CH):
                        y = _dot_nt(h, w[c * CH:(c + 1) * CH, :]).astype(BF16)
                        dst[pl.ds(j * nb, nb), :, c * CH:(c + 1) * CH] = y.reshape(nb, TB, CH)
            if first:
                copies[2].wait()
                copies[3].wait()

            ns.__exit__(None, None, None); ns = jax.named_scope("rec"); ns.__enter__()
            j0 = nj - WARM
            sel = (_iota((NC * M, R), 0) // M == _iota((NC * M, R), 1) // seg).astype(BF16)
            vt = vall[(j0 - 1) * nb:j0 * nb].reshape(R, HD)
            g = (_dot(sel, vt) * (1.0 / (M + seg))).astype(BF16)
            mems[...] = jnp.zeros_like(mems)
            mems[j0] = _dot(g, wob[...]).astype(BF16)

            qr, kc = _iota((MB, KB), 0), _iota((MB, KB), 1)
            mem_mask = qr // M == jnp.where(kc < TB, kc // seg, (kc - TB) // M)

            def step(st):
                j, n, _ = st

                @pl.when(j == 0)
                def _():
                    ends = mems[nj].astype(F32)
                    mems[0] = jnp.concatenate(
                        [mem0_ref[...].astype(F32), ends[:(NC - 1) * M]], axis=0).astype(BF16)

                m = mems[j]
                blocks = pl.ds(j * nb, nb)
                new, pend = None, None
                for p in range(npair + 1):
                    prev = pend
                    if p < npair:
                        lanes = slice(p * PW, (p + 1) * PW)
                        km = _dot_nt(m, wk[lanes, :]).astype(BF16).reshape(nb, MB, PW)
                        q = _dot_nt(m, wq[lanes, :])
                        vm = _dot_nt(m, wv[lanes, :]).astype(BF16).reshape(nb, MB, PW)
                        kmem[blocks, :, lanes] = km
                        vmem[blocks, :, lanes] = vm
                        pend = attend(q, kall, vall, km, vm, j, lanes, mem_mask), lanes
                    if prev is not None:
                        y = _dot(prev[0](), wob[prev[1], :])
                        new = y if new is None else new + y
                new = new.astype(BF16)
                bits = lambda a: pltpu.bitcast(a.astype(F32), jnp.int32)
                differs = jnp.max((bits(new) != bits(mems[j + 1])).astype(jnp.int32))
                mems[j + 1] = new
                done = (differs == 0) & (n >= WARM + nj - 1)
                return jnp.where(j == nj - 1, 0, j + 1), n + 1, done.astype(jnp.int32)

            lax.while_loop(lambda st: (st[2] == 0) & (st[1] < WARM + NC * nj), step,
                           (jnp.int32(j0), jnp.int32(0), jnp.int32(0)))

            ns.__exit__(None, None, None); ns = jax.named_scope("tok"); ns.__enter__()
            qr, kc = _iota((TB, KB), 0), _iota((TB, KB), 1)
            tok_mask = ((qr // seg == jnp.where(kc < TB, kc // seg, (kc - TB) // M))
                        & ((qr >= kc) | (kc >= TB)))

            @pl.loop(0, nj)
            def _(j):
                r = pl.ds(pl.multiple_of(j * R, R), R)

                pend = None
                for p in range(npair + 1):
                    prev = pend
                    if p < npair:
                        lanes = slice(p * PW, (p + 1) * PW)
                        q = _dot_nt(hs[r, :], wq[lanes, :])
                        pend = attend(q, kall, vall, kmem[pl.ds(j * nb, nb), :, lanes],
                                      vmem[pl.ds(j * nb, nb), :, lanes], j, lanes, tok_mask), lanes
                    if prev is not None:
                        xs[r, :] += _dot(prev[0](), wob[prev[1], :])
            ns.__exit__(None, None, None)

        pl.run_scoped(body,
                      pltpu.VMEM((nj * nb, TB, HD), BF16), pltpu.VMEM((nj * nb, TB, HD), BF16),
                      pltpu.VMEM((nj + 1, NC * M, D), BF16),
                      pltpu.VMEM((nj * nb, MB, HD), BF16), pltpu.VMEM((nj * nb, MB, HD), BF16))

    for layer in range(2):
        with jax.named_scope("ln"):
            layernorm()
        with jax.named_scope("A"):
            layer_a()
        with jax.named_scope("ln"):
            layernorm()
        layer_b(layer == 0)

    @pl.loop(0, nseg)
    def _(i):
        mine, orig = seg_rows(i)
        out_ref[orig, :] = xs[mine, :].astype(out_ref.dtype)


@functools.partial(jax.jit, static_argnames=("B_seg_len",))
def pallas_interleave_layers__linear_kernel_hedgehog__memory_aug_recurrent_mem_tr__prompt_kernel(
    A_x, A_wqkv, A_w_phi, A_wo, B_x, B_mem0, B_Wq, B_Wk, B_Wv, B_Wo, B_seg_len,
):
    del B_x
    Bn, S, D = A_x.shape
    assert Bn == 1
    H, dhb = B_Wq.shape[1:]
    dha = D // HA
    phit = jnp.broadcast_to(A_w_phi.reshape(D, dha).T[None, :, None, :],
                            (HA // 8, dha, 8, D)).reshape(D, D)
    vmem = pl.BlockSpec(memory_space=pltpu.VMEM)
    hbm = pl.BlockSpec(memory_space=pl.ANY)
    out = pl.pallas_call(
        functools.partial(_kernel, seg=B_seg_len, dhb=dhb),
        out_shape=jax.ShapeDtypeStruct((S, D), A_x.dtype),
        in_specs=[vmem] * 5 + [hbm] * 4,
        out_specs=vmem,
        scratch_shapes=[
            pltpu.VMEM((S, D), F32), pltpu.VMEM((S, D), BF16),
            pltpu.VMEM((H * dhb, D), BF16), pltpu.VMEM((H * dhb, D), BF16),
            pltpu.VMEM((H * dhb, D), BF16), pltpu.VMEM((H * dhb, D), BF16),
            pltpu.VMEM((D, D), BF16), pltpu.VMEM((D, D), BF16), pltpu.VMEM((D, D), BF16),
            pltpu.SemaphoreType.DMA((4,)),
        ],
        compiler_params=pltpu.CompilerParams(vmem_limit_bytes=127 * 2**20),
    )(A_x.reshape(S, D), A_wqkv, phit, A_wo, B_mem0.reshape(-1, D),
      B_Wq.reshape(D, H * dhb).T, B_Wk.reshape(D, H * dhb).T, B_Wv.reshape(D, H * dhb).T,
      B_Wo.reshape(H * dhb, D))
    return out.reshape(Bn, S, D)
```
